```python
import jax
import jax.numpy as jnp

def _softmax(x, axis=-1):
    return jax.nn.softmax(x, axis=axis)

def _gelu(x):
    return jax.nn.gelu(x, approximate=True)

def _silu(x):
    return jax.nn.silu(x)

def _sigmoid(x):
    return jax.nn.sigmoid(x)

def _layernorm(x, axis=-1, eps=1e-05):
    m = jnp.mean(x, axis=axis, keepdims=True)
    v = jnp.var(x, axis=axis, keepdims=True)
    return (x - m) / jnp.sqrt(v + eps)

def _scatter_add(tgt, idx, src, axis=0):
    return tgt.at[idx].add(src)

def _segment_sum(src, seg, n):
    return jax.ops.segment_sum(src, seg, n)

class _Rng:

    def __init__(self, key):
        self._k = key

    def _next(self):
        self._k, sub = jax.random.split(self._k)
        return sub

    def normal(self, shape):
        return jax.random.normal(self._next(), shape, dtype=jnp.bfloat16)

    def randint(self, lo, hi, shape):
        return jax.random.randint(self._next(), shape, lo, hi, dtype=jnp.int32)

    def uniform(self, shape, lo=0.0, hi=1.0):
        return jax.random.uniform(self._next(), shape, jnp.bfloat16, lo, hi)

    def permutation(self, n):
        return jax.random.permutation(self._next(), n)
kernel_name = 'concat_heads__compressed_kv_cla__memory_aug_recurrent_mem_tr__prompt'

def setup_inputs():
    _rng = _Rng(jax.random.key(int.from_bytes(__import__("os").urandom(4), "little")))
    _w = lambda a: (lambda t: t.astype(jnp.bfloat16) if jnp.issubdtype(t.dtype, jnp.floating) else t)(jnp.asarray(a))

    def _A_setup():
        B, H, Sq, Sk, D, M = (1, 32, 2048, 2048, 128, 576)
        Dc = 4 * D
        return {'x': _w((lambda *s: _rng.normal(s) * 0.05)(B, Sq, M)), 'c_kv': _w((lambda *s: _rng.normal(s) * 0.05)(B, Sk, Dc)), 'w_q': _w((lambda *s: _rng.normal(s) * 0.05)(M, H, D) * M ** (-0.5)), 'w_uk': _w((lambda *s: _rng.normal(s) * 0.05)(Dc, H, D) * Dc ** (-0.5)), 'w_uv': _w((lambda *s: _rng.normal(s) * 0.05)(Dc, H, D) * Dc ** (-0.5)), 'w_o': _w((lambda *s: _rng.normal(s) * 0.05)(H, D, M) * (H * D) ** (-0.5))}
    _A_in = _A_setup()

    def _B_setup():
        B, S, Dm = (1, 2048, 576)
        H, Dh = (32, 128)
        M, seg = (8, 32)
        seg = min(seg, S)
        S = S // seg * seg
        return {'x': _w((lambda *s: _rng.normal(s) * 0.05)(B, S, Dm)), 'mem0': _w((lambda *s: _rng.normal(s) * 0.05)(B, M, Dm)), 'Wq': _w((lambda *s: _rng.normal(s) * 0.05)(Dm, H, Dh) * Dm ** (-0.5)), 'Wk': _w((lambda *s: _rng.normal(s) * 0.05)(Dm, H, Dh) * Dm ** (-0.5)), 'Wv': _w((lambda *s: _rng.normal(s) * 0.05)(Dm, H, Dh) * Dm ** (-0.5)), 'Wo': _w((lambda *s: _rng.normal(s) * 0.05)(H, Dh, Dm) * (H * Dh) ** (-0.5)), 'seg_len': seg}
    _B_in = _B_setup()
    return {'A_x': _A_in['x'], 'A_c_kv': _A_in['c_kv'], 'A_w_q': _A_in['w_q'], 'A_w_uk': _A_in['w_uk'], 'A_w_uv': _A_in['w_uv'], 'A_w_o': _A_in['w_o'], 'B_x': _B_in['x'], 'B_mem0': _B_in['mem0'], 'B_Wq': _B_in['Wq'], 'B_Wk': _B_in['Wk'], 'B_Wv': _B_in['Wv'], 'B_Wo': _B_in['Wo'], 'B_seg_len': _B_in['seg_len']}

def reference(A_x, A_c_kv, A_w_q, A_w_uk, A_w_uv, A_w_o, B_x, B_mem0, B_Wq, B_Wk, B_Wv, B_Wo, B_seg_len):

    def _A_ref(x, c_kv, w_q, w_uk, w_uv, w_o):
        B, Sq, M = (x.shape[0], x.shape[1], x.shape[2])
        Sk = c_kv.shape[1]
        H, D = (w_q.shape[1], w_q.shape[2])
        q = jnp.einsum('bqm,mhd->bhqd', x, w_q)
        k = jnp.einsum('bkc,chd->bhkd', c_kv, w_uk)
        v = jnp.einsum('bkc,chd->bhkd', c_kv, w_uv)
        scores = jnp.einsum('bhqd,bhkd->bhqk', q, k) * D ** (-0.5)
        off = Sk - Sq
        qi = jnp.arange(Sq)[:, None]
        kj = jnp.arange(Sk)[None, :]
        cmask = kj <= qi + off
        scores = jnp.where(cmask[None, None], scores, -1000000000.0)
        p = _softmax(scores, axis=-1)
        ctx = jnp.einsum('bhqk,bhkd->bhqd', p, v)
        return jnp.einsum('bhqd,hdm->bqm', ctx, w_o)

    def _B_ref(x, mem0, Wq, Wk, Wv, Wo, seg_len):
        B, S, Dm = x.shape
        H, Dh = (Wq.shape[1], Wq.shape[2])
        M = mem0.shape[1]
        scale = Dh ** (-0.5)
        n_seg = S // seg_len
        L = M + seg_len
        idx = jnp.arange(L)
        mask = (idx[:, None] < M) | (idx[:, None] >= idx[None, :])
        mem = mem0
        outs = []
        for s in range(n_seg):
            xs = x[:, s * seg_len:(s + 1) * seg_len, :].copy()
            h = jnp.concatenate([mem, xs], axis=1)
            q = jnp.einsum('btd,dhe->bhte', h, Wq)
            k = jnp.einsum('btd,dhe->bhte', h, Wk)
            v = jnp.einsum('btd,dhe->bhte', h, Wv)
            scores = jnp.einsum('bhqe,bhke->bhqk', q, k) * scale
            scores = jnp.where(mask[None, None], scores, -1000000000.0)
            p = _softmax(scores, axis=-1)
            o = jnp.einsum('bhqk,bhke->bhqe', p, v)
            o = jnp.einsum('bhte,hed->btd', o, Wo)
            mem = o[:, :M, :].copy()
            outs.append(o[:, M:, :])
        return jnp.concatenate(outs, axis=1)
    a = _A_ref(A_x, A_c_kv, A_w_q, A_w_uk, A_w_uv, A_w_o)
    b = _B_ref(B_x, B_mem0, B_Wq, B_Wk, B_Wv, B_Wo, B_seg_len)
    return jnp.concatenate([a, b], axis=-1)
```

```python
import functools
import numpy as np
import jax
import jax.numpy as jnp
from jax import lax
from jax.experimental import pallas as pl
from jax.experimental.pallas import tpu as pltpu

F32 = jnp.float32
BF16 = jnp.bfloat16
LOG2E = 1.4426950408889634
BQ = 128

def _nt(a, b):
    return lax.dot_general(a, b, (((1,), (1,)), ((), ())), preferred_element_type=F32)
def _nn(a, b):
    return jnp.dot(a, b, preferred_element_type=F32)
def _rb(x):
    return x.astype(BF16).astype(F32)

def make_kernel(S, H, D, DM, DC, seg, M, do_a, do_b):
    nq = S // BQ
    nseg = S // seg
    L = M + seg
    HD = H * D
    scale = float(D) ** -0.5 * LOG2E
    G = 128 // L
    groups = [(g0, min(G, H - g0)) for g0 in range(0, H, G)]
    NG = len(groups)

    def kernel(xa_h, c_h, wq_h, wuk_h, wuv_h, wo_h, xb_h, mem0_h, bq_h, bk_h, bv_h, bo_h, out_h,
               xa, c, wo, xb, mem0, bo, xa_t, xb_t, bo2, raw, w2, q_scr, k_scr, v_scr, acc, out, sems, osem):
        HH = H // 2
        ws = [(wq_h, DM), (wuk_h, DC), (wuv_h, DC)]
        wb = [(bq_h, DM), (bk_h, DM), (bv_h, DM)]
        order = [(w, k, 0) for w, k in ws] + [(w, k, 1) for w, k in ws] + [(w, k, j) for w, k in wb for j in range(2)]
        offs = np.cumsum([0] + [k for _, k, _ in order]).tolist()
        wc = [pltpu.make_async_copy(w.at[:, pl.ds(j*HH, HH), :], raw.at[pl.ds(offs[i], k)], sems.at[i]) for i, (w, k, j) in enumerate(order)]
        oc = [pltpu.make_async_copy(s_, d_, sems.at[12+i]) for i, (s_, d_) in enumerate([(xa_h, xa_t), (c_h, c), (wo_h, wo), (xb_h, xb_t), (mem0_h, mem0), (bo_h, bo)])]
        def relay(r0, n):
            w2[pl.ds(r0, n), :] = raw[pl.ds(r0, n)].reshape(n, HH * D)
        oc[0].start(); wc[0].start()
        acc[...] = jnp.zeros_like(acc)
        oc[0].wait()
        oc[1].start(); wc[1].start()
        xa[...] = xa_t[...].T
        wc[0].wait()
        wc[2].start()
        relay(0, DM)
        oc[1].wait(); wc[1].wait()
        oc[2].start()
        relay(offs[1], DC)
        wc[2].wait()
        for i in range(3, 6):
            wc[i].start()
        relay(offs[2], DC)
        oc[2].wait()
        for i in range(6, 12):
            wc[i].start()
        for i in range(3, 6):
            oc[i].start()
        UR = 176
        del_rows = offs[3] - UR
        def filler(h):
            r0 = pl.multiple_of(jnp.minimum(del_rows + h * UR, offs[12] - UR), 16)
            relay(r0, UR)
        hA = 1
        hB = (offs[6] - del_rows) // UR
        assert (offs[6] - del_rows - 1) // UR < HH and del_rows + H * UR >= offs[12]
        rows = lax.broadcasted_iota(jnp.int32, (BQ, BQ), 0)
        cols = lax.broadcasted_iota(jnp.int32, (BQ, BQ), 1)
        causal = cols <= rows

        def qk(i):
            kend = (i + 1) * BQ
            return _nt(q_scr[i*BQ:kend, :], k_scr[0:kend, :])
        def sm(s, i):
            sd = jnp.where(causal, s[:, i*BQ:], -1e30)
            s = jnp.concatenate([s[:, :i*BQ], sd], axis=1) if i > 0 else sd
            m = jnp.max(s, axis=1, keepdims=True)
            p = jnp.exp2(s - m)
            l = jnp.sum(p, axis=1, keepdims=True)
            return p.astype(BF16), pl.reciprocal(l, approx=False)
        def pv(h, p, r, i):
            kend = (i + 1) * BQ
            o = _nn(p, v_scr[0:kend, :]) * r
            acc[i*BQ:kend, :] += _nt(o.astype(BF16), wo[h])
        def head(h, _):
            @pl.when(h == hA)
            def _():
                for i in range(3, 6):
                    wc[i].wait()
            @pl.when(h == hB)
            def _():
                for i in range(6, 12):
                    wc[i].wait()
            hs = pl.ds(pl.multiple_of((h % HH) * D, D), D)
            hi = h // HH
            def wsl(i, k):
                return w2[pl.ds(pl.multiple_of(offs[i] + hi * offs[3], 16), k), hs]
            q_scr[...] = (_nn(xa[...], wsl(0, DM)) * scale).astype(BF16)
            cv = c[...]
            k_scr[...] = _nn(cv, wsl(1, DC)).astype(BF16)
            v_scr[...] = _nn(cv, wsl(2, DC)).astype(BF16)
            s = qk(0)
            for i in range(nq):
                sn = qk(i + 1) if i + 1 < nq else None
                if i == 8:
                    filler(h)
                p, r = sm(s, i)
                pv(h, p, r, i)
                s = sn
            return 0
        if do_a:
            lax.fori_loop(0, H, head, 0)
        out[:, 0:DM] = acc[...].astype(BF16)

        for i in range(3, 6):
            oc[i].wait()
        xb[...] = xb_t[...].T
        for hh in range(H):
            bo2[hh*D:(hh+1)*D, :] = bo[hh].T
        def bw(m, g0, n):
            parts = []
            for j in range(2):
                lo, hi_ = max(g0, j*HH), min(g0+n, (j+1)*HH)
                if hi_ > lo:
                    o_ = offs[6 + 2*m + j]
                    parts.append(w2[o_:o_+DM, (lo-j*HH)*D:(hi_-j*HH)*D])
            return parts[0] if len(parts) == 1 else jnp.concatenate(parts, axis=1)
        r = lax.broadcasted_iota(jnp.int32, (G*L, G*L), 0)
        cc = lax.broadcasted_iota(jnp.int32, (G*L, G*L), 1)
        def blk(z):
            hz = jnp.zeros_like(z)
            for g in range(1, G):
                hz = hz + (z >= g * L).astype(jnp.int32)
            return hz, z - hz * L
        hr, pr = blk(r)
        hc, pc = blk(cc)
        mask = (hr == hc) & ((pr < M) | (pr >= pc))
        def stack(a, n):
            return jnp.concatenate([a[:, j*D:(j+1)*D] for j in range(n)], axis=0)
        def unstack(a, n):
            return jnp.concatenate([a[j*L:(j+1)*L, :] for j in range(n)], axis=1)
        def b_proj(h, g):
            g0, n = groups[g]
            sl = slice(g0*D, (g0+n)*D)
            q = stack(_nn(h, bw(0, g0, n)), n)
            k = stack(_nn(h, bw(1, g0, n)), n)
            v = stack(_nn(h, bw(2, g0, n)), n)
            return (_rb(q) * scale).astype(BF16), k.astype(BF16), v.astype(BF16)
        def b_sm(sc, g):
            n = groups[g][1]
            sc = jnp.where(mask[:n*L, :n*L], sc, -1e30)
            mx = jnp.max(sc, axis=1, keepdims=True)
            p = jnp.exp2(sc - mx)
            l = jnp.sum(p, axis=1, keepdims=True)
            return (p * pl.reciprocal(l, approx=False)).astype(BF16)
        def b_wo(o, g):
            g0, n = groups[g]
            return _nn(o, bo2[g0*D:(g0+n)*D, :])
        def step(s, mem):
            r0 = pl.multiple_of(s * seg, seg)
            xs = xb[pl.ds(r0, seg), :].astype(F32)
            h = jnp.concatenate([mem, xs], axis=0)
            a = None
            qkv = {}; sc = {}; o = {}; p = {}
            for t in range(NG + 4):
                if t < NG: qkv[t] = b_proj(h, t)
                if 0 <= t-1 < NG: sc[t-1] = _nt(qkv[t-1][0], qkv[t-1][1])
                if 0 <= t-2 < NG: p[t-2] = b_sm(sc[t-2], t-2)
                if 0 <= t-3 < NG: o[t-3] = unstack(_rb(_nn(p[t-3], qkv[t-3][2])), groups[t-3][1])
                if 0 <= t-4 < NG:
                    w = b_wo(o[t-4], t-4)
                    a = w if a is None else a + w
            res = a.astype(BF16)
            out[pl.ds(r0, seg), DM:2*DM] = res[M:, :]
            return res[0:M, :].astype(F32)
        NCH = 4
        per = nseg // NCH
        ocps = [pltpu.make_async_copy(out.at[pl.ds(j*per*seg, per*seg)], out_h.at[pl.ds(j*per*seg, per*seg)], osem.at[j]) for j in range(NCH)]
        if do_b:
            mem = mem0[...].astype(F32)
            def outer(j, mem):
                mem = lax.fori_loop(j*per, (j+1)*per, step, mem)
                r0 = pl.multiple_of(j*per*seg, per*seg)
                pltpu.make_async_copy(out.at[pl.ds(r0, per*seg)], out_h.at[pl.ds(r0, per*seg)], osem.at[j]).start()
                return mem
            lax.fori_loop(0, NCH, outer, mem)
        else:
            out[:, DM:] = jnp.zeros((S, DM), BF16)
            for o_ in ocps:
                o_.start()
        for o_ in ocps:
            o_.wait()
    return kernel

def run(A_x, A_c_kv, A_w_q, A_w_uk, A_w_uv, A_w_o, B_x, B_mem0, B_Wq, B_Wk, B_Wv, B_Wo, B_seg_len, do_a=True, do_b=True, interpret=False):
    _, S, DM = A_x.shape
    H, D = A_w_q.shape[1], A_w_q.shape[2]
    DC = A_c_kv.shape[2]
    M = B_mem0.shape[1]
    seg = int(B_seg_len)
    kern = make_kernel(S, H, D, DM, DC, seg, M, do_a, do_b)
    V = pltpu.VMEM
    RT = 2 * (4 * DM + 2 * DC)
    scratch = [
        V((S, DM), BF16), V((S, DC), BF16), V((H, DM, D), BF16), V((S, DM), BF16), V((M, DM), BF16), V((H, DM, D), BF16),
        V((DM, S), BF16), V((DM, S), BF16), V((H*D, DM), BF16), V((RT, H//2, D), BF16), V((RT, H//2*D), BF16),
        V((S, D), BF16), V((S, D), BF16), V((S, D), BF16), V((S, DM), F32), V((S, 2*DM), BF16),
        pltpu.SemaphoreType.DMA((18,)), pltpu.SemaphoreType.DMA((4,)),
    ]
    out = pl.pallas_call(
        kern, out_shape=jax.ShapeDtypeStruct((S, 2*DM), BF16),
        in_specs=[pl.BlockSpec(memory_space=pl.ANY)] * 12, out_specs=pl.BlockSpec(memory_space=pl.ANY),
        scratch_shapes=scratch,
        compiler_params=pltpu.CompilerParams(vmem_limit_bytes=120*1024*1024),
        name="fused", interpret=interpret,
    )(A_x[0].T, A_c_kv[0], A_w_q, A_w_uk, A_w_uv, jnp.swapaxes(A_w_o, 1, 2), B_x[0].T, B_mem0[0], B_Wq, B_Wk, B_Wv, jnp.swapaxes(B_Wo, 1, 2))
    return out.reshape(1, S, 2*DM)


@functools.partial(jax.jit, static_argnames=("B_seg_len",))
def pallas_concat_heads__compressed_kv_cla__memory_aug_recurrent_mem_tr__prompt_kernel(
    A_x, A_c_kv, A_w_q, A_w_uk, A_w_uv, A_w_o, B_x, B_mem0, B_Wq, B_Wk, B_Wv, B_Wo, B_seg_len,
):
    return run(A_x, A_c_kv, A_w_q, A_w_uk, A_w_uv, A_w_o, B_x, B_mem0, B_Wq, B_Wk, B_Wv, B_Wo, B_seg_len)
```

```python
import functools
import numpy as np
import jax
import jax.numpy as jnp
from jax import lax
from jax.experimental import pallas as pl
from jax.experimental.pallas import tpu as pltpu

F32 = jnp.float32
BF16 = jnp.bfloat16
LOG2E = 1.4426950408889634
BQ = 128

def _nt(a, b):
    return lax.dot_general(a, b, (((1,), (1,)), ((), ())), preferred_element_type=F32)
def _nn(a, b):
    return jnp.dot(a, b, preferred_element_type=F32)
def _rb(x):
    return x.astype(BF16).astype(F32)

def make_kernel(S, H, D, DM, DC, seg, M, do_a, do_b):
    nq = S // BQ
    nseg = S // seg
    L = M + seg
    HD = H * D
    scale = float(D) ** -0.5 * LOG2E
    G = 128 // L
    groups = [(g0, min(G, H - g0)) for g0 in range(0, H, G)]
    NG = len(groups)

    def kernel(xa_h, c_h, wq_h, wuk_h, wuv_h, wo_h, xb_h, mem0_h, bq_h, bk_h, bv_h, bo_h, out_h,
               xa, c, wo, xb, mem0, bo, xa_t, xb_t, bo2, raw, w2, q_scr, k_scr, v_scr, acc, out, sems, osem):
        HH = H // 2
        ws = [(wq_h, DM), (wuk_h, DC), (wuv_h, DC)]
        wb = [(bq_h, DM), (bk_h, DM), (bv_h, DM)]
        order = [(w, k, 0) for w, k in ws] + [(w, k, 1) for w, k in ws] + [(w, k, j) for w, k in wb for j in range(2)]
        offs = np.cumsum([0] + [k for _, k, _ in order]).tolist()
        wc = [pltpu.make_async_copy(w.at[:, pl.ds(j*HH, HH), :], raw.at[pl.ds(offs[i], k)], sems.at[i]) for i, (w, k, j) in enumerate(order)]
        oc = [pltpu.make_async_copy(s_, d_, sems.at[12+i]) for i, (s_, d_) in enumerate([(xa_h, xa_t), (c_h, c), (wo_h, wo), (xb_h, xb_t), (mem0_h, mem0), (bo_h, bo)])]
        def relay(r0, n):
            w2[pl.ds(r0, n), :] = raw[pl.ds(r0, n)].reshape(n, HH * D)
        oc[0].start(); wc[0].start()
        acc[...] = jnp.zeros_like(acc)
        oc[0].wait()
        oc[1].start(); wc[1].start()
        xa[...] = xa_t[...].T
        wc[0].wait()
        wc[2].start()
        relay(0, DM)
        oc[1].wait(); wc[1].wait()
        oc[2].start()
        relay(offs[1], DC)
        wc[2].wait()
        for i in range(3, 6):
            wc[i].start()
        relay(offs[2], DC)
        oc[2].wait()
        for i in range(6, 12):
            wc[i].start()
        for i in range(3, 6):
            oc[i].start()
        UR = 176
        del_rows = offs[3] - UR
        def filler(h):
            r0 = pl.multiple_of(jnp.minimum(del_rows + h * UR, offs[12] - UR), 16)
            relay(r0, UR)
        hA = 1
        hB = (offs[6] - del_rows) // UR
        assert (offs[6] - del_rows - 1) // UR < HH and del_rows + H * UR >= offs[12]
        rows = lax.broadcasted_iota(jnp.int32, (BQ, BQ), 0)
        cols = lax.broadcasted_iota(jnp.int32, (BQ, BQ), 1)
        causal = cols <= rows

        def qk(i):
            kend = (i + 1) * BQ
            return _nt(q_scr[i*BQ:kend, :], k_scr[0:kend, :])
        def sm(s, i):
            sd = jnp.where(causal, s[:, i*BQ:], -1e30)
            s = jnp.concatenate([s[:, :i*BQ], sd], axis=1) if i > 0 else sd
            m = jnp.max(s, axis=1, keepdims=True)
            p = jnp.exp2(s - m)
            l = jnp.sum(p, axis=1, keepdims=True)
            return p.astype(BF16), pl.reciprocal(l, approx=False)
        def pv(h, p, r, i):
            kend = (i + 1) * BQ
            o = _nn(p, v_scr[0:kend, :]) * r
            acc[i*BQ:kend, :] += _nt(o.astype(BF16), wo[h])
        def head(h, _):
            @pl.when(h == hA)
            def _():
                for i in range(3, 6):
                    wc[i].wait()
            @pl.when(h == hB)
            def _():
                for i in range(6, 12):
                    wc[i].wait()
            hs = pl.ds(pl.multiple_of((h % HH) * D, D), D)
            hi = h // HH
            def wsl(i, k):
                return w2[pl.ds(pl.multiple_of(offs[i] + hi * offs[3], 16), k), hs]
            q_scr[...] = (_nn(xa[...], wsl(0, DM)) * scale).astype(BF16)
            cv = c[...]
            k_scr[...] = _nn(cv, wsl(1, DC)).astype(BF16)
            v_scr[...] = _nn(cv, wsl(2, DC)).astype(BF16)
            s = qk(0)
            for i in range(nq):
                sn = qk(i + 1) if i + 1 < nq else None
                if i == 8:
                    filler(h)
                p, r = sm(s, i)
                pv(h, p, r, i)
                s = sn
            return 0
        if do_a:
            lax.fori_loop(0, H, head, 0)
        out[:, 0:DM] = acc[...].astype(BF16)

        for i in range(3, 6):
            oc[i].wait()
        xb[...] = xb_t[...].T
        for hh in range(H):
            bo2[hh*D:(hh+1)*D, :] = bo[hh].T
        def bw(m, g0, n):
            parts = []
            for j in range(2):
                lo, hi_ = max(g0, j*HH), min(g0+n, (j+1)*HH)
                if hi_ > lo:
                    o_ = offs[6 + 2*m + j]
                    parts.append(w2[o_:o_+DM, (lo-j*HH)*D:(hi_-j*HH)*D])
            return parts[0] if len(parts) == 1 else jnp.concatenate(parts, axis=1)
        r = lax.broadcasted_iota(jnp.int32, (G*L, G*L), 0)
        cc = lax.broadcasted_iota(jnp.int32, (G*L, G*L), 1)
        def blk(z):
            hz = jnp.zeros_like(z)
            for g in range(1, G):
                hz = hz + (z >= g * L).astype(jnp.int32)
            return hz, z - hz * L
        hr, pr = blk(r)
        hc, pc = blk(cc)
        mask = (hr == hc) & ((pr < M) | (pr >= pc))
        def stack(a, n):
            return jnp.concatenate([a[:, j*D:(j+1)*D] for j in range(n)], axis=0)
        def unstack(a, n):
            return jnp.concatenate([a[j*L:(j+1)*L, :] for j in range(n)], axis=1)
        def b_proj(h, g):
            g0, n = groups[g]
            sl = slice(g0*D, (g0+n)*D)
            q = stack(_nn(h, bw(0, g0, n)), n)
            k = stack(_nn(h, bw(1, g0, n)), n)
            v = stack(_nn(h, bw(2, g0, n)), n)
            return (_rb(q) * scale).astype(BF16), k.astype(BF16), v.astype(BF16)
        def b_sm(sc, g):
            n = groups[g][1]
            sc = jnp.where(mask[:n*L, :n*L], sc, -1e30)
            mx = jnp.max(sc, axis=1, keepdims=True)
            p = jnp.exp2(sc - mx)
            l = jnp.sum(p, axis=1, keepdims=True)
            return (p * pl.reciprocal(l, approx=False)).astype(BF16)
        def b_wo(o, g):
            g0, n = groups[g]
            return _nn(o, bo2[g0*D:(g0+n)*D, :])
        def step(s, mem):
            r0 = pl.multiple_of(s * seg, seg)
            xs = xb[pl.ds(r0, seg), :].astype(F32)
            h = jnp.concatenate([mem, xs], axis=0)
            a = None
            qkv = {}; sc = {}; o = {}; p = {}
            for t in range(NG + 6):
                if t < NG: qkv[t] = b_proj(h, t)
                if 0 <= t-1 < NG: sc[t-1] = _nt(qkv[t-1][0], qkv[t-1][1])
                if 0 <= t-2 < NG: p[t-2] = b_sm(sc[t-2], t-2)
                if 0 <= t-3 < NG: o[t-3] = unstack(_rb(_nn(p[t-3], qkv[t-3][2])), groups[t-3][1])
                if 0 <= t-6 < NG:
                    w = b_wo(o[t-6], t-6)
                    a = w if a is None else a + w
            res = a.astype(BF16)
            out[pl.ds(r0, seg), DM:2*DM] = res[M:, :]
            return res[0:M, :].astype(F32)
        NCH = 4
        per = nseg // NCH
        ocps = [pltpu.make_async_copy(out.at[pl.ds(j*per*seg, per*seg)], out_h.at[pl.ds(j*per*seg, per*seg)], osem.at[j]) for j in range(NCH)]
        if do_b:
            mem = mem0[...].astype(F32)
            def outer(j, mem):
                mem = lax.fori_loop(0, per//2, lambda u, m_: step(j*per+2*u+1, step(j*per+2*u, m_)), mem)
                r0 = pl.multiple_of(j*per*seg, per*seg)
                pltpu.make_async_copy(out.at[pl.ds(r0, per*seg)], out_h.at[pl.ds(r0, per*seg)], osem.at[j]).start()
                return mem
            lax.fori_loop(0, NCH, outer, mem)
        else:
            out[:, DM:] = jnp.zeros((S, DM), BF16)
            for o_ in ocps:
                o_.start()
        for o_ in ocps:
            o_.wait()
    return kernel

def run(A_x, A_c_kv, A_w_q, A_w_uk, A_w_uv, A_w_o, B_x, B_mem0, B_Wq, B_Wk, B_Wv, B_Wo, B_seg_len, do_a=True, do_b=True, interpret=False):
    _, S, DM = A_x.shape
    H, D = A_w_q.shape[1], A_w_q.shape[2]
    DC = A_c_kv.shape[2]
    M = B_mem0.shape[1]
    seg = int(B_seg_len)
    kern = make_kernel(S, H, D, DM, DC, seg, M, do_a, do_b)
    V = pltpu.VMEM
    RT = 2 * (4 * DM + 2 * DC)
    scratch = [
        V((S, DM), BF16), V((S, DC), BF16), V((H, DM, D), BF16), V((S, DM), BF16), V((M, DM), BF16), V((H, DM, D), BF16),
        V((DM, S), BF16), V((DM, S), BF16), V((H*D, DM), BF16), V((RT, H//2, D), BF16), V((RT, H//2*D), BF16),
        V((S, D), BF16), V((S, D), BF16), V((S, D), BF16), V((S, DM), F32), V((S, 2*DM), BF16),
        pltpu.SemaphoreType.DMA((18,)), pltpu.SemaphoreType.DMA((4,)),
    ]
    out = pl.pallas_call(
        kern, out_shape=jax.ShapeDtypeStruct((S, 2*DM), BF16),
        in_specs=[pl.BlockSpec(memory_space=pl.ANY)] * 12, out_specs=pl.BlockSpec(memory_space=pl.ANY),
        scratch_shapes=scratch,
        compiler_params=pltpu.CompilerParams(vmem_limit_bytes=120*1024*1024),
        name="fused", interpret=interpret,
    )(A_x[0].T, A_c_kv[0], A_w_q, A_w_uk, A_w_uv, jnp.swapaxes(A_w_o, 1, 2), B_x[0].T, B_mem0[0], B_Wq, B_Wk, B_Wv, jnp.swapaxes(B_Wo, 1, 2))
    return out.reshape(1, S, 2*DM)


@functools.partial(jax.jit, static_argnames=("B_seg_len",))
def pallas_concat_heads__compressed_kv_cla__memory_aug_recurrent_mem_tr__prompt_kernel(
    A_x, A_c_kv, A_w_q, A_w_uk, A_w_uv, A_w_o, B_x, B_mem0, B_Wq, B_Wk, B_Wv, B_Wo, B_seg_len,
):
    return run(A_x, A_c_kv, A_w_q, A_w_uk, A_w_uv, A_w_o, B_x, B_mem0, B_Wq, B_Wk, B_Wv, B_Wo, B_seg_len)
```
